```python
import os as _os
_os.environ.setdefault("JAX_PLATFORMS", "cpu")
import jax
import jax.numpy as jnp

def _softmax(x, axis=-1):
    return jax.nn.softmax(x, axis=axis)
def _gelu(x):
    return jax.nn.gelu(x, approximate=True)
def _silu(x):
    return jax.nn.silu(x)
def _sigmoid(x):
    return jax.nn.sigmoid(x)
def _layernorm(x, axis=-1, eps=1e-5):
    m = jnp.mean(x, axis=axis, keepdims=True)
    v = jnp.var(x, axis=axis, keepdims=True)
    return (x - m) / jnp.sqrt(v + eps)
def _scatter_add(tgt, idx, src, axis=0):
    return tgt.at[idx].add(src)
def _segment_sum(src, seg, n):
    return jax.ops.segment_sum(src, seg, n)
class _Rng:
    def __init__(self, key):
        self._k = key
    def _next(self):
        self._k, sub = jax.random.split(self._k)
        return sub
    def normal(self, shape):
        return jax.random.normal(self._next(), shape, dtype=jnp.bfloat16)
    def randint(self, lo, hi, shape):
        return jax.random.randint(self._next(), shape, lo, hi, dtype=jnp.int32)
    def uniform(self, shape, lo=0.0, hi=1.0):
        return jax.random.uniform(self._next(), shape, jnp.bfloat16, lo, hi)
    def permutation(self, n):
        return jax.random.permutation(self._next(), n)


kernel_name = 'interleave_layers__mha_block__dense_activation_mish__prompt'

def setup_inputs():
    _rng = _Rng(jax.random.key(int.from_bytes(__import__("os").urandom(4), "little")))
    _w = (lambda a: (lambda t: t.astype(jnp.bfloat16) if jnp.issubdtype(t.dtype, jnp.floating) else t)(jnp.asarray(a)))
    def _A_setup():
        B, S, D, H = 1, 2048, 512, 32
        return {
            "x": _w((lambda *s: _rng.normal(s) * 0.05)(B, S, D)),
            "wqkv": _w((lambda *s: _rng.normal(s) * 0.05)(D, 3 * D)),
            "wo": _w((lambda *s: _rng.normal(s) * 0.05)(D, D)),
        }
    _A_in = _A_setup()

    def _B_setup():
        B, S, D, F = 1, 2048, 512, 1792
        return {
            "x": _w((lambda *s: _rng.normal(s) * 0.05)(B, S, D)),
            "w1": _w((lambda *s: _rng.normal(s) * 0.4)(D, F) * (D ** -0.5)),
            "b1": _w((lambda *s: _rng.normal(s) * 0.4)(F)),
            "w2": _w((lambda *s: _rng.normal(s) * 0.4)(F, D) * (F ** -0.5)),
        }
    _B_in = _B_setup()

    return {
        "A_x": _A_in["x"],
        "A_wqkv": _A_in["wqkv"],
        "A_wo": _A_in["wo"],
        "B_x": _B_in["x"],
        "B_w1": _B_in["w1"],
        "B_b1": _B_in["b1"],
        "B_w2": _B_in["w2"],
    }

def reference(A_x, A_wqkv, A_wo, B_x, B_w1, B_b1, B_w2):
    def _A_ref(x, wqkv, wo):
        B, S, D = x.shape
        H = 32
        Dh = D // H
        qkv = (lambda x, *d: x.transpose(*d))((x @ wqkv).reshape(B, S, 3, H, Dh), 2, 0, 3, 1, 4)
        q, k, v = qkv[0], qkv[1], qkv[2]
        scores = jnp.einsum("bhqd,bhkd->bhqk", q, k) * (Dh ** -0.5)
        p = _softmax(scores, axis=-1)
        o = jnp.einsum("bhqk,bhkd->bhqd", p, v)
        return (lambda x, *d: x.transpose(*d))(o, 0, 2, 1, 3).reshape(B, S, D) @ wo

    def _B_ref(x, w1, b1, w2):
        h = jnp.einsum("bsd,df->bsf", x, w1) + b1
        sp = jnp.log1p(jnp.exp(-jnp.abs(h))) + jnp.where(h > 0, h, jnp.zeros_like(h))
        act = h * jnp.tanh(sp)
        return jnp.einsum("bsf,fd->bsd", act, w2)

    x = A_x
    x = x + _A_ref(_layernorm(x, axis=-1), A_wqkv, A_wo)
    x = x + _B_ref(_layernorm(x, axis=-1), B_w1, B_b1, B_w2)
    x = x + _A_ref(_layernorm(x, axis=-1), A_wqkv, A_wo)
    x = x + _B_ref(_layernorm(x, axis=-1), B_w1, B_b1, B_w2)
    return x
```

```python
import math

import jax
import jax.numpy as jnp
import jax.experimental.pallas as pl
import jax.experimental.pallas.tpu as pltpu

S = 2048
D = 512
H = 32
DH = D // H
F = 1792
NLAYERS = 2

TQ = 1024
CK = 128
NJ = S // TQ
NC = S // CK
NIT = H * NJ
RC = 256
EPS = 1e-5
QSCALE = (DH ** -0.5) * math.log2(math.e)

_NT = (((1,), (1,)), ((), ()))
_TN = (((0,), (0,)), ((), ()))


def _layernorm(x):
    m = jnp.mean(x, axis=-1, keepdims=True)
    xc = x - m
    v = jnp.mean(xc * xc, axis=-1, keepdims=True)
    return xc * jax.lax.rsqrt(v + EPS)


def _mish(h):
    sp = jnp.log1p(jnp.exp(-jnp.abs(h))) + jnp.maximum(h, 0.0)
    return h * jnp.tanh(sp)


def _kernel(x_ref, wqkv_ref, wo_ref, w1_ref, b1_ref, w2_ref, o_ref,
            xs_ref, xn_ref, wqt_ref, wvt_ref, k_ref, qt_ref, vt_ref, ot_ref,
            s0_ref, s1_ref):
    f32 = jnp.float32
    bf16 = jnp.bfloat16

    xs_ref[...] = x_ref[...].astype(f32)
    wqt_ref[...] = wqkv_ref[:, 0:D].T
    wvt_ref[...] = wqkv_ref[:, 2 * D:3 * D].T

    def prep_a(idx):
        h = idx // NJ
        j = idx % NJ
        g = h // 8
        r = h % 8
        qt = qt_ref[j, pl.ds(pl.multiple_of(g * 128, 128), 128), :]
        row = jax.lax.broadcasted_iota(jnp.int32, (128, TQ), 0)
        qtm = jnp.where((row >> 4) == r, qt, jnp.zeros_like(qt))
        return g, qtm

    def chunk_a(g, qtm, c, s_ref, mrun):
        kblk = k_ref[g, pl.ds(c * CK, CK), :]
        s = jnp.dot(kblk, qtm, preferred_element_type=f32)
        s_ref[pl.ds(c * CK, CK), :] = s
        mc = jnp.max(s.reshape(CK // 8, 8, TQ), axis=0)
        return mc if mrun is None else jnp.maximum(mrun, mc)

    def chunk_b(h, c, s_ref, m, acc):
        p = jnp.exp2(s_ref[pl.ds(c * CK, CK), :] - m).astype(bf16)
        vt = vt_ref[pl.ds(pl.multiple_of(h * DH, DH), DH), pl.ds(c * CK, CK)]
        vta = jnp.concatenate([vt, jnp.ones((DH, CK), bf16)], axis=0)
        o = jnp.dot(vta, p, preferred_element_type=f32)
        return o if acc is None else acc + o

    def both(idx_a, sa_ref, idx_b, sb_ref, m_b):
        g, qtm = prep_a(idx_a)
        hb = idx_b // NJ
        jb = idx_b % NJ
        mrun = None
        acc = None
        for c in range(NC):
            mrun = chunk_a(g, qtm, c, sa_ref, mrun)
            acc = chunk_b(hb, c, sb_ref, m_b, acc)
        ot_ref[jb, pl.ds(pl.multiple_of(hb * DH, DH), DH), :] = (
            acc[:DH] / acc[DH:]).astype(bf16)
        return jnp.max(mrun, axis=0, keepdims=True)

    def layer(_, carry):
        for rc in range(S // RC):
            rows = pl.ds(rc * RC, RC)
            xn_ref[rows, :] = _layernorm(xs_ref[rows, :]).astype(bf16)
        for rc in range(S // 512):
            rows = pl.ds(rc * 512, 512)
            xn = xn_ref[rows, :]
            kk = jnp.dot(xn, wqkv_ref[:, D:2 * D],
                         preferred_element_type=f32).astype(bf16)
            for g in range(4):
                k_ref[g, rows, :] = kk[:, g * 128:(g + 1) * 128]
            qt = jax.lax.dot_general(wqt_ref[...], xn, _NT,
                                     preferred_element_type=f32)
            j = (rc * 512) // TQ
            off = (rc * 512) % TQ
            qt_ref[j, :, pl.ds(off, 512)] = (qt * QSCALE).astype(bf16)
            vt = jax.lax.dot_general(wvt_ref[...], xn, _NT,
                                     preferred_element_type=f32)
            vt_ref[:, rows] = vt.astype(bf16)

        g, qtm = prep_a(0)
        mrun = None
        for c in range(NC):
            mrun = chunk_a(g, qtm, c, s0_ref, mrun)
        m0 = jnp.max(mrun, axis=0, keepdims=True)

        def body(it, m0):
            i = 2 * it
            m1 = both(i + 1, s1_ref, i, s0_ref, m0)
            nxt = jnp.minimum(i + 2, NIT - 1)
            return both(nxt, s0_ref, i + 1, s1_ref, m1)

        jax.lax.fori_loop(0, NIT // 2, body, m0)

        for rc in range(S // 512):
            rows = pl.ds(rc * 512, 512)
            j = (rc * 512) // TQ
            off = (rc * 512) % TQ
            att = jax.lax.dot_general(ot_ref[j, :, pl.ds(off, 512)], wo_ref[...],
                                      _TN, preferred_element_type=f32)
            xs_ref[rows, :] += att

        for rc in range(S // RC):
            rows = pl.ds(rc * RC, RC)
            x = xs_ref[rows, :]
            xn = _layernorm(x).astype(bf16)
            h = jnp.dot(xn, w1_ref[...], preferred_element_type=f32)
            h = h + b1_ref[...].astype(f32)
            act = _mish(h).astype(bf16)
            y = jnp.dot(act, w2_ref[...], preferred_element_type=f32)
            xs_ref[rows, :] = x + y
        return carry

    jax.lax.fori_loop(0, NLAYERS, layer, 0)
    o_ref[...] = xs_ref[...].astype(o_ref.dtype)


@jax.jit
def pallas_interleave_layers__mha_block__dense_activation_mish__prompt_kernel(
    A_x: jax.Array,
    A_wqkv: jax.Array,
    A_wo: jax.Array,
    B_x: jax.Array,
    B_w1: jax.Array,
    B_b1: jax.Array,
    B_w2: jax.Array,
):
    del B_x
    x = A_x.reshape(S, D)
    b1 = B_b1.reshape(1, F)
    bf16 = jnp.bfloat16
    out = pl.pallas_call(
        _kernel,
        out_shape=jax.ShapeDtypeStruct((S, D), A_x.dtype),
        scratch_shapes=[
            pltpu.VMEM((S, D), jnp.float32),
            pltpu.VMEM((S, D), bf16),
            pltpu.VMEM((D, D), bf16),
            pltpu.VMEM((D, D), bf16),
            pltpu.VMEM((4, S, 128), bf16),
            pltpu.VMEM((NJ, D, TQ), bf16),
            pltpu.VMEM((D, S), bf16),
            pltpu.VMEM((NJ, D, TQ), bf16),
            pltpu.VMEM((S, TQ), jnp.float32),
            pltpu.VMEM((S, TQ), jnp.float32),
        ],
        compiler_params=pltpu.CompilerParams(
            vmem_limit_bytes=100 * 1024 * 1024),
    )(x, A_wqkv, A_wo, B_w1, b1, B_w2)
    return out.reshape(A_x.shape)
```

```python
import math

import jax
import jax.numpy as jnp
import jax.experimental.pallas as pl
import jax.experimental.pallas.tpu as pltpu

S = 2048
D = 512
H = 32
DH = D // H
F = 1792
NLAYERS = 2

TQ = 512
CK = 128
SK = 3
LAG = 2
LAGL = 1
UNROLL = 14
NJ = S // TQ
NC = S // CK
NIT = H * NJ
RC = 256
EPS = 1e-5
QSCALE = (DH ** -0.5) * math.log2(math.e)

_NT = (((1,), (1,)), ((), ()))
_TN = (((0,), (0,)), ((), ()))


def _layernorm(x):
    m = jnp.mean(x, axis=-1, keepdims=True)
    xc = x - m
    v = jnp.mean(xc * xc, axis=-1, keepdims=True)
    return xc * jax.lax.rsqrt(v + EPS)


def _mish(h):
    sp = jnp.log1p(jnp.exp(-jnp.abs(h))) + jnp.maximum(h, 0.0)
    return h * jnp.tanh(sp)


def _kernel(x_ref, wqkv_ref, wo_hbm, w1_hbm, b1_ref, w2_hbm, o_hbm,
            xs_ref, xn_ref, wt_ref, qt_ref, kt_ref, vt_ref, ot_ref,
            s0_ref, s1_ref, wo_ref, w1_ref, w2_ref, ob_ref, wsem, osem):
    f32 = jnp.float32
    bf16 = jnp.bfloat16

    w_copies = [
        pltpu.make_async_copy(wo_hbm, wo_ref, wsem.at[0]),
        pltpu.make_async_copy(w1_hbm, w1_ref, wsem.at[1]),
        pltpu.make_async_copy(w2_hbm, w2_ref, wsem.at[2]),
    ]
    for cp in w_copies:
        cp.start()

    def out_copy(rc):
        rows = pl.ds(rc * RC, RC)
        return pltpu.make_async_copy(ob_ref.at[rows, :], o_hbm.at[rows, :],
                                     osem.at[rc])

    xs_ref[...] = x_ref[...].astype(f32)
    wt_ref[...] = wqkv_ref[...].T

    def tie(m8, deps):
        mi = pltpu.bitcast(m8, jnp.int32)
        for d in deps:
            di = pltpu.bitcast(d, jnp.int32)
            mi = jnp.maximum(mi, jnp.minimum(mi, di))
        return pltpu.bitcast(mi, f32)

    def head_rows(h):
        return pl.ds(pl.multiple_of(h * DH, DH), DH)

    def prep_a(idx):
        h = idx // NJ
        j = idx % NJ
        return h, qt_ref[j, head_rows(h), :]

    def chunk_a(h, qt, c, s_ref, mrun):
        kt = kt_ref[head_rows(h), pl.ds(c * CK, CK)]
        s = jax.lax.dot_general(kt, qt, _TN, preferred_element_type=f32)
        s_ref[pl.ds(c * CK, CK), :] = s
        mc = jnp.max(s.reshape(CK // 8, 8, TQ), axis=0)
        return mc if mrun is None else jnp.maximum(mrun, mc)

    def chunk_b(h, c, s_ref, m8, acc, lrun):
        pf = jnp.exp2(s_ref[pl.ds(c * CK, CK), :].reshape(CK // 8, 8, TQ)
                      - m8[None])
        lc = jnp.sum(pf, axis=0)
        p = pf.reshape(CK, TQ).astype(bf16)
        vt = vt_ref[head_rows(h), pl.ds(c * CK, CK)]
        o = jnp.dot(vt, p, preferred_element_type=f32)
        return (o if acc is None else acc + o,
                lc if lrun is None else lrun + lc)

    def finish(i, acc, lrun):
        l = jnp.sum(lrun, axis=0, keepdims=True)
        ot_ref[i % NJ, head_rows(i // NJ), :] = (acc / l).astype(bf16)

    def col_max(mrun):
        return jnp.broadcast_to(jnp.max(mrun, axis=0, keepdims=True), (8, TQ))

    def both(i, s_cur, s_oth, carry, first=False, last=False):
        m_prev, m_cur, acc, lrun = carry
        if not last:
            ha, qt = prep_a(i + 1)
        hp = (i - 1) // NJ
        hc = i // NJ
        mrun = None
        lsave = None
        hist = []
        for c in range(NC):
            u = c - SK
            deps = ((hist[c - LAG][0],) if c >= LAG else ()) + (
                (hist[c - LAGL][1],) if c >= LAGL else ())
            deps = tuple(d for d in deps if d is not None)
            if u < 0:
                if not first:
                    acc, lrun = chunk_b(hp, u + NC, s_oth, tie(m_prev, deps),
                                        acc, lrun)
                    lsave = lrun
                    if u == -1:
                        finish(i - 1, acc, lrun)
                if u == -1:
                    acc = None
                    lrun = None
            if not last:
                mrun = chunk_a(ha, qt, c, s_oth, mrun)
            if u >= 0:
                acc, lrun = chunk_b(hc, u, s_cur, tie(m_cur, deps), acc, lrun)
                lsave = lrun
            hist.append((mrun, lsave))
        if last:
            for u in range(NC - SK, NC):
                acc, lrun = chunk_b(hc, u, s_cur, m_cur, acc, lrun)
            finish(i, acc, lrun)
            return None
        return (m_cur, col_max(mrun), acc, lrun)

    def layer(li, carry):
        for rc in range(S // RC):
            rows = pl.ds(rc * RC, RC)
            xn_ref[rows, :] = _layernorm(xs_ref[rows, :]).astype(bf16)
        for j in range(NJ):
            rows = pl.ds(j * TQ, TQ)
            xn = xn_ref[rows, :]
            qt = jax.lax.dot_general(wt_ref[0:D, :], xn, _NT,
                                     preferred_element_type=f32)
            qt_ref[j] = (qt * QSCALE).astype(bf16)
            kt = jax.lax.dot_general(wt_ref[D:2 * D, :], xn, _NT,
                                     preferred_element_type=f32)
            kt_ref[:, rows] = kt.astype(bf16)
            vt = jax.lax.dot_general(wt_ref[2 * D:3 * D, :], xn, _NT,
                                     preferred_element_type=f32)
            vt_ref[:, rows] = vt.astype(bf16)

        h0, qt0 = prep_a(0)
        mrun = None
        for c in range(NC):
            mrun = chunk_a(h0, qt0, c, s0_ref, mrun)
        m0 = col_max(mrun)
        st = both(0, s0_ref, s1_ref, (m0, m0, None, None), first=True)

        def body(it, st):
            i = UNROLL * it + 1
            for t in range(0, UNROLL, 2):
                st = both(i + t, s1_ref, s0_ref, st)
                st = both(i + t + 1, s0_ref, s1_ref, st)
            return st

        @pl.when(li == 0)
        def _():
            for cp in w_copies:
                cp.wait()

        nb = (NIT - 2) // UNROLL
        st = jax.lax.fori_loop(0, nb, body, st)
        for i in range(UNROLL * nb + 1, NIT - 1, 2):
            st = both(i, s1_ref, s0_ref, st)
            st = both(i + 1, s0_ref, s1_ref, st)
        both(NIT - 1, s1_ref, s0_ref, st, last=True)

        for j in range(NJ):
            rows = pl.ds(j * TQ, TQ)
            att = jax.lax.dot_general(ot_ref[j], wo_ref[...], _TN,
                                      preferred_element_type=f32)
            xs_ref[rows, :] += att

        for rc in range(S // RC):
            rows = pl.ds(rc * RC, RC)
            x = xs_ref[rows, :]
            xn = _layernorm(x).astype(bf16)
            h = jnp.dot(xn, w1_ref[...], preferred_element_type=f32)
            h = h + b1_ref[...].astype(f32)
            act = _mish(h).astype(bf16)
            y = jnp.dot(act, w2_ref[...], preferred_element_type=f32)
            xnew = x + y
            xs_ref[rows, :] = xnew
            ob_ref[rows, :] = xnew.astype(ob_ref.dtype)

            @pl.when(li == NLAYERS - 1)
            def _():
                out_copy(rc).start()
        return carry

    jax.lax.fori_loop(0, NLAYERS, layer, 0)
    for rc in range(S // RC):
        out_copy(rc).wait()


@jax.jit
def pallas_interleave_layers__mha_block__dense_activation_mish__prompt_kernel(
    A_x: jax.Array,
    A_wqkv: jax.Array,
    A_wo: jax.Array,
    B_x: jax.Array,
    B_w1: jax.Array,
    B_b1: jax.Array,
    B_w2: jax.Array,
):
    del B_x
    x = A_x.reshape(S, D)
    b1 = B_b1.reshape(1, F)
    bf16 = jnp.bfloat16
    out = pl.pallas_call(
        _kernel,
        out_shape=jax.ShapeDtypeStruct((S, D), A_x.dtype),
        in_specs=[
            pl.BlockSpec(memory_space=pltpu.VMEM),
            pl.BlockSpec(memory_space=pltpu.VMEM),
            pl.BlockSpec(memory_space=pl.ANY),
            pl.BlockSpec(memory_space=pl.ANY),
            pl.BlockSpec(memory_space=pltpu.VMEM),
            pl.BlockSpec(memory_space=pl.ANY),
        ],
        out_specs=pl.BlockSpec(memory_space=pl.ANY),
        scratch_shapes=[
            pltpu.VMEM((S, D), jnp.float32),
            pltpu.VMEM((S, D), bf16),
            pltpu.VMEM((3 * D, D), bf16),
            pltpu.VMEM((NJ, D, TQ), bf16),
            pltpu.VMEM((D, S), bf16),
            pltpu.VMEM((D, S), bf16),
            pltpu.VMEM((NJ, D, TQ), bf16),
            pltpu.VMEM((S, TQ), jnp.float32),
            pltpu.VMEM((S, TQ), jnp.float32),
            pltpu.VMEM((D, D), bf16),
            pltpu.VMEM((D, F), bf16),
            pltpu.VMEM((F, D), bf16),
            pltpu.VMEM((S, D), A_x.dtype),
            pltpu.SemaphoreType.DMA((3,)),
            pltpu.SemaphoreType.DMA((S // RC,)),
        ],
        compiler_params=pltpu.CompilerParams(
            vmem_limit_bytes=100 * 1024 * 1024),
    )(x, A_wqkv, A_wo, B_w1, b1, B_w2)
    return out.reshape(A_x.shape)
```
